```python
import os as _os
_os.environ.setdefault("JAX_PLATFORMS", "cpu")
import jax
import jax.numpy as jnp

def _softmax(x, axis=-1):
    return jax.nn.softmax(x, axis=axis)
def _gelu(x):
    return jax.nn.gelu(x, approximate=True)
def _silu(x):
    return jax.nn.silu(x)
def _sigmoid(x):
    return jax.nn.sigmoid(x)
def _layernorm(x, axis=-1, eps=1e-5):
    m = jnp.mean(x, axis=axis, keepdims=True)
    v = jnp.var(x, axis=axis, keepdims=True)
    return (x - m) / jnp.sqrt(v + eps)
def _scatter_add(tgt, idx, src, axis=0):
    return tgt.at[idx].add(src)
def _segment_sum(src, seg, n):
    return jax.ops.segment_sum(src, seg, n)
class _Rng:
    def __init__(self, key):
        self._k = key
    def _next(self):
        self._k, sub = jax.random.split(self._k)
        return sub
    def normal(self, shape):
        return jax.random.normal(self._next(), shape, dtype=jnp.bfloat16)
    def randint(self, lo, hi, shape):
        return jax.random.randint(self._next(), shape, lo, hi, dtype=jnp.int32)
    def uniform(self, shape, lo=0.0, hi=1.0):
        return jax.random.uniform(self._next(), shape, jnp.bfloat16, lo, hi)
    def permutation(self, n):
        return jax.random.permutation(self._next(), n)


kernel_name = 'sequential_preLN__sliding_block__dense_activation_gelu__prompt'

def setup_inputs():
    _rng = _Rng(jax.random.key(int.from_bytes(__import__("os").urandom(4), "little")))
    _w = (lambda a: (lambda t: t.astype(jnp.bfloat16) if jnp.issubdtype(t.dtype, jnp.floating) else t)(jnp.asarray(a)))
    def _A_setup():
        B, S, D = 1, 2048, 640
        return {
            "x": _w((lambda *s: _rng.normal(s) * 0.05)(B, S, D)),
            "wqkv": _w((lambda *s: _rng.normal(s) * 0.05)(D, 3 * D)),
            "wo": _w((lambda *s: _rng.normal(s) * 0.05)(D, D)),
        }
    _A_in = _A_setup()

    def _B_setup():
        B, S, D, F = 1, 2048, 640, 1536
        return {
            "x": _w((lambda *s: _rng.normal(s) * 0.05)(B, S, D)),
            "w1": _w((lambda *s: _rng.normal(s) * 0.8)(D, F) * (D ** -0.5)),
            "b1": _w((lambda *s: _rng.normal(s) * 0.8)(F) * 0.01),
            "w2": _w((lambda *s: _rng.normal(s) * 0.8)(F, D) * (F ** -0.5)),
            "b2": _w((lambda *s: _rng.normal(s) * 0.05)(D) * 0.01),
        }
    _B_in = _B_setup()

    return {
        "A_x": _A_in["x"],
        "A_wqkv": _A_in["wqkv"],
        "A_wo": _A_in["wo"],
        "B_x": _B_in["x"],
        "B_w1": _B_in["w1"],
        "B_b1": _B_in["b1"],
        "B_w2": _B_in["w2"],
        "B_b2": _B_in["b2"],
    }

def reference(A_x, A_wqkv, A_wo, B_x, B_w1, B_b1, B_w2, B_b2):
    def _A_ref(x, wqkv, wo):
        B, S, D = x.shape
        H = 32; Dh = D // H; W = 256
        qkv = (lambda x, *d: x.transpose(*d))((x @ wqkv).reshape(B, S, 3, H, Dh), 2, 0, 3, 1, 4)
        q, k, v = qkv[0], qkv[1], qkv[2]
        scores = jnp.einsum("bhqd,bhkd->bhqk", q, k) * (Dh ** -0.5)
        idx = jnp.arange(S)
        mask = (idx[:, None] - idx[None, :] >= 0) & (idx[:, None] - idx[None, :] < W)
        scores = jnp.where(mask[None, None], scores, -1e9)
        p = _softmax(scores, axis=-1)
        o = jnp.einsum("bhqk,bhkd->bhqd", p, v)
        return (lambda x, *d: x.transpose(*d))(o, 0, 2, 1, 3).reshape(B, S, D) @ wo

    def _B_ref(x, w1, b1, w2, b2):
        h = jnp.einsum("bsd,df->bsf", x, w1) + b1
        h = _gelu(h)
        return jnp.einsum("bsf,fd->bsd", h, w2) + b2

    x = A_x
    h = x + _A_ref(_layernorm(x, axis=-1), A_wqkv, A_wo)
    h2 = h + _B_ref(_layernorm(h, axis=-1), B_w1, B_b1, B_w2, B_b2)
    return h2
```

```python
import functools

import jax
import jax.numpy as jnp
import numpy as np
from jax import lax
from jax.experimental import pallas as pl
from jax.experimental.pallas import tpu as pltpu

_H = 32
_W = 256
_TQ = 256
_QB = 64
_NG = 16
_GB = 4
_LAG = 1
_EPS = 1e-5
_F32 = jnp.float32
_BF16 = jnp.bfloat16
_NT = (((1,), (1,)), ((), ()))
_NN = (((1,), (0,)), ((), ()))


def _dot(a, b, dims=_NN):
    return lax.dot_general(a, b, dims, preferred_element_type=_F32)


def _layernorm(x):
    m = jnp.mean(x, axis=-1, keepdims=True)
    c = x - m
    v = jnp.mean(c * c, axis=-1, keepdims=True)
    return c * lax.rsqrt(v + _EPS)


def _as_i32(x):
    return pltpu.bitcast(x, jnp.int32)


def _as_bf16(x):
    return pltpu.bitcast(x, _BF16)


def _combine_tiles(t):
    tiles = [t[:, 128 * c:128 * (c + 1)] for c in range(5)]
    lane = lax.broadcasted_iota(jnp.int32, tiles[0].shape, 1)
    out = []
    for m in range(8):
        spans = []
        for f0 in (40 * m, 40 * m + 320):
            c, l0 = divmod(f0, 128)
            spans.append((c, l0, min(l0 + 40, 128)))
            if l0 + 40 > 128:
                spans.append((c + 1, 0, l0 + 40 - 128))
        spans.sort(key=lambda sp: sp[1])
        acc = tiles[spans[0][0]]
        for c, l0, _ in spans[1:]:
            acc = jnp.where(lane >= l0, tiles[c], acc)
        out.append(acc)
    return out


def _attention(q_scr, k_scr, vt_scr, s_scr, step, dh, first):
    lane_q = lax.broadcasted_iota(jnp.int32, (_QB // 2, 128), 1)
    row = lax.broadcasted_iota(jnp.int32, (_QB, 128), 0)
    col = lax.broadcasted_iota(jnp.int32, (_QB, 128), 1) & (_QB - 1)
    causal = row <= col
    low8 = lax.broadcasted_iota(jnp.int32, (8, 128), 1) < 64
    top4 = lax.broadcasted_iota(jnp.int32, (8, 128), 0) < 4
    low64 = lax.broadcasted_iota(jnp.int32, (64, 128), 1) < 64
    low128 = lax.broadcasted_iota(jnp.int32, (128, 128), 1) < 64
    zeros = jnp.zeros((_QB, 128), _F32)
    nslot = s_scr.shape[0]
    batches = [(j, b) for j in range(_TQ // _QB) for b in range(_NG // _GB)]
    maxes, d0, d1, outs = {}, {}, {}, []

    def scores(n):
        j, b = batches[n]
        for m in range(b * _GB // 2, (b + 1) * _GB // 2):
            q = _as_i32(q_scr[j * _QB:(j + 1) * _QB, 128 * m:128 * (m + 1)])
            parts = []
            for f0 in (40 * m, 40 * m + 64, 40 * m + dh, 40 * m + 64 + dh):
                parts.append(jnp.where(((lane_q - f0) & 127) < dh, q, 0))
            wq = _as_bf16(jnp.concatenate(parts, axis=0))
            if first:
                nk = _QB * (j + 1)
                kw = k_scr[0:nk, 128 * m:128 * (m + 1)]
            else:
                r0 = pl.multiple_of(step * _TQ + (j * _QB - _W), _QB)
                kw = k_scr[pl.ds(r0, _W + _QB), 128 * m:128 * (m + 1)]
            s2 = _dot(kw, wq, _NT)
            for e in range(2):
                g = 2 * m + e
                s = s2[:, 128 * e:128 * (e + 1)]
                if first:
                    diag = jnp.where(causal, s[nk - _QB:], -1e30)
                    s = jnp.concatenate([s[:nk - _QB], diag], axis=0) if j else diag
                else:
                    s = jnp.concatenate(
                        [s[_QB:_W], jnp.where(causal, s[_W:], s[:_QB])], axis=0)
                s_scr[n % nslot, g % _GB, 0:s.shape[0]] = s
                maxes[j, g] = jnp.max(s, axis=0, keepdims=True)

    def values(n):
        j, b = batches[n]
        for g in range(b * _GB, (b + 1) * _GB):
            nk = _QB * (j + 1) if first else _W
            p = jnp.exp2(s_scr[n % nslot, g % _GB, 0:nk] - maxes[j, g])
            if first:
                if j % 2 == 0:
                    p = jnp.concatenate([p, zeros], axis=0)
                tile0, ntile = 0, j // 2 + 1
            else:
                mid, mer = p[:_W - _QB], p[_W - _QB:]
                pieces = [jnp.where(causal, 0.0, mer), mid, jnp.where(causal, mer, 0.0)]
                p = jnp.concatenate(
                    pieces + [zeros] if j % 2 == 0 else [zeros] + pieces, axis=0)
                tile0, ntile = step * (_TQ // 128) + (j // 2 - _W // 128), 3
            vt = jnp.concatenate(
                [vt_scr[tile0 + c, 48 * g:48 * (g + 1), :] for c in range(ntile)], axis=1)
            r = _dot(vt, p.astype(_BF16))
            ra, rb = r[:24], r[24:]
            lv, lr = (16, 4) if g % 2 == 0 else (0, 0)
            inv = 1.0 / jnp.where(low8, ra[lv:lv + 8], rb[lv:lv + 8])[lr:lr + 1]
            d0[j, g] = ra * inv
            d1[j, g] = rb * inv
        if b == _NG // _GB - 1:
            def stack(dd):
                rows = []
                for g in range(0, _NG, 2):
                    e, o = dd[j, g], dd[j, g + 1]
                    rows += [e[:16], jnp.where(top4, e[16:], o[:8]), o[8:]]
                return jnp.concatenate(rows, axis=0)

            s0, s1 = stack(d0), stack(d1)
            x1 = jnp.where(low128, s0[0:128], s1[64:192]).astype(_BF16).T
            x2 = jnp.where(low128, s0[128:256], s1[192:320]).astype(_BF16).T
            x3 = jnp.concatenate([s0[256:320], s1[0:64]], axis=0).T
            x3 = jnp.where(low64, x3[:_QB], x3[_QB:]).astype(_BF16)
            outs.append(jnp.concatenate(
                [x1[:_QB], x2[:_QB], x3, x1[_QB:], x2[_QB:]], axis=1))

    for n in range(len(batches) + _LAG):
        if n < len(batches):
            scores(n)
        if n >= _LAG:
            values(n - _LAG)
    return jnp.concatenate(outs, axis=0)


def _kernel(x_ref, wqkv_hbm, wo_hbm, w1_hbm, b1_ref, w2_hbm, b2_ref, o_ref,
            wqkv, wvt, wo, w1, w2, q_scr, k_scr, vt_scr, s_scr, att_scr, sems):
    step = pl.program_id(0)
    d = x_ref.shape[-1]
    dh = d // _H
    copies = [pltpu.make_async_copy(src, dst, sems.at[n]) for n, (src, dst) in enumerate(
        [(wqkv_hbm, wqkv), (wo_hbm, wo), (w1_hbm, w1), (w2_hbm, w2)])]

    @pl.when(step == 0)
    def _():
        for c in copies:
            c.start()
        copies[0].wait()
        wvt[...] = wqkv[:, 2 * d:].T

    x = x_ref[...].astype(_F32)
    xn = _layernorm(x).astype(_BF16)

    rows = pl.ds(pl.multiple_of(step * _TQ, _TQ), _TQ)
    k_tiles = _combine_tiles(_dot(xn, wqkv[:, d:2 * d]))
    for t, kt in enumerate(k_tiles):
        k_scr[rows, 128 * t:128 * (t + 1)] = kt.astype(_BF16)

    vt = _dot(wvt[...], xn, _NT)
    top4 = lax.broadcasted_iota(jnp.int32, (8, _TQ), 0) < 4
    pieces = []
    for g in range(_NG):
        for b in range(2):
            base = (g // 2) * 2 * dh + b * (d // 2)
            if g % 2 == 0:
                pieces += [vt[base:base + 16], jnp.where(top4, vt[base + 16:base + 24], 1.0)]
            else:
                pieces += [jnp.where(top4, 1.0, vt[base + 16:base + 24]), vt[base + 24:base + 40]]
    vtp = jnp.concatenate(pieces, axis=0).astype(_BF16)
    for c in range(_TQ // 128):
        vt_scr[step * (_TQ // 128) + c] = vtp[:, 128 * c:128 * (c + 1)]

    scale = float(dh ** -0.5 * np.log2(np.e))
    for t, qt in enumerate(_combine_tiles(_dot(xn, wqkv[:, :d]) * scale)):
        q_scr[:, 128 * t:128 * (t + 1)] = qt.astype(_BF16)

    @pl.when(step == 0)
    def _():
        att_scr[...] = _attention(q_scr, k_scr, vt_scr, s_scr, step, dh, True)
        for c in copies[1:]:
            c.wait()

    @pl.when(step > 0)
    def _():
        att_scr[...] = _attention(q_scr, k_scr, vt_scr, s_scr, step, dh, False)

    h = x + _dot(att_scr[...], wo[...])
    hn = _layernorm(h).astype(_BF16)
    a = _dot(hn, w1[...]) + b1_ref[...].astype(_F32).reshape(1, -1)
    a = jax.nn.gelu(a, approximate=True).astype(_BF16)
    o_ref[...] = (h + _dot(a, w2[...]) + b2_ref[...].astype(_F32).reshape(1, -1)).astype(o_ref.dtype)


@jax.jit
def pallas_sequential_preLN__sliding_block__dense_activation_gelu__prompt_kernel(
    A_x: jax.Array,
    A_wqkv: jax.Array,
    A_wo: jax.Array,
    B_x: jax.Array,
    B_w1: jax.Array,
    B_b1: jax.Array,
    B_w2: jax.Array,
    B_b2: jax.Array,
):
    del B_x
    b, s, d = A_x.shape
    f = B_w1.shape[1]
    assert b == 1 and d == 640 and s % _TQ == 0
    hbm = pl.BlockSpec(memory_space=pl.ANY)
    out = pl.pallas_call(
        _kernel,
        grid=(s // _TQ,),
        in_specs=[
            pl.BlockSpec((_TQ, d), lambda i: (i, 0)),
            hbm, hbm, hbm,
            pl.BlockSpec((f,), lambda i: (0,)),
            hbm,
            pl.BlockSpec((d,), lambda i: (0,)),
        ],
        out_specs=pl.BlockSpec((_TQ, d), lambda i: (i, 0)),
        out_shape=jax.ShapeDtypeStruct((s, d), A_x.dtype),
        scratch_shapes=[
            pltpu.VMEM((d, 3 * d), _BF16),
            pltpu.VMEM((d, d), _BF16),
            pltpu.VMEM((d, d), _BF16),
            pltpu.VMEM((d, f), _BF16),
            pltpu.VMEM((f, d), _BF16),
            pltpu.VMEM((_TQ, 8 * 128), _BF16),
            pltpu.VMEM((s, 8 * 128), _BF16),
            pltpu.VMEM((s // 128, 48 * _NG, 128), _BF16),
            pltpu.VMEM((_LAG + 1, _GB, _W, 128), _F32),
            pltpu.VMEM((_TQ, d), _BF16),
            pltpu.SemaphoreType.DMA((4,)),
        ],
        compiler_params=pltpu.CompilerParams(
            dimension_semantics=("arbitrary",),
            vmem_limit_bytes=100 * 1024 * 1024,
        ),
    )(A_x.reshape(s, d), A_wqkv, A_wo, B_w1, B_b1, B_w2, B_b2)
    return out.reshape(b, s, d)
```

```python
import jax
import jax.numpy as jnp
import numpy as np
from jax import lax
from jax.experimental import pallas as pl
from jax.experimental.pallas import tpu as pltpu

_H = 32
_W = 256
_TQ = 256
_QB = 32
_GB = 2
_LAG = 4
_FC = 512
_HALO = 96
_EPS = 1e-5
_MASKED = -1e30
_F32 = jnp.float32
_BF16 = jnp.bfloat16
_NT = (((1,), (1,)), ((), ()))
_NN = (((1,), (0,)), ((), ()))


def _dot(a, b, dims=_NN):
    return lax.dot_general(a, b, dims, preferred_element_type=_F32)


def _gelu2(x):
    c = float(np.sqrt(2.0 / np.pi))
    return x * jnp.tanh(x * (x * x * (0.044715 * c) + c)) + x


def _layernorm(x):
    m = jnp.mean(x, axis=-1, keepdims=True)
    c = x - m
    v = jnp.mean(c * c, axis=-1, keepdims=True)
    return c * lax.rsqrt(v + _EPS)


def _as_i32(x):
    return pltpu.bitcast(x, jnp.int32)


def _as_bf16(x):
    return pltpu.bitcast(x, _BF16)


def _pack_rows(x):
    bits = lax.bitcast_convert_type(x, jnp.int32) + 0x8000
    lo = jnp.concatenate([bits[r:r + 8] for r in range(0, x.shape[0], 16)], axis=0)
    hi = jnp.concatenate([bits[r + 8:r + 16] for r in range(0, x.shape[0], 16)], axis=0)
    return lax.shift_right_logical(lo, 16) | (hi & -65536)


def _head_tiles(t):
    tiles = [t[:, 128 * c:128 * (c + 1)] for c in range(5)]
    lane = lax.broadcasted_iota(jnp.int32, (1, 128), 1)
    return ([tiles[0]]
            + [jnp.where(lane >= 128 - 8 * m, tiles[m - 1], tiles[m]) for m in range(1, 5)]
            + [tiles[4]])


def _aligned(i, n):
    return i if isinstance(i, int) else pl.multiple_of(i, n)


def _attention(q_scr, ks_scr, vt_scr, mask_scr, s_scr, att_scr, step, dh, first):
    hb = _QB // 2
    row = lax.broadcasted_iota(jnp.int32, (_QB, 128), 0)
    lane = lax.broadcasted_iota(jnp.int32, (_QB, 128), 1)
    col = lane & (_QB - 1)
    causal = row <= col
    prow = (row[:hb] & 7) + 2 * (row[:hb] & 8)
    new_bits = (jnp.where(prow <= col[:hb], 0xFFFF, 0)
                | jnp.where(prow + 8 <= col[:hb], -65536, 0))
    odd = (lane[:hb] & 32) != 0
    upper = lane[:hb] >= 64
    top4 = lax.broadcasted_iota(jnp.int32, (8, 128), 0) < 4
    zero = jnp.zeros((hb, 128), jnp.int32)
    nslot = s_scr.shape[0]
    stages = [(u, b) for u in range(_TQ // 128) for b in range(_H // _GB)]
    maxes, outs = {}, {}

    def first_block(u):
        return 5 - 4 * u if first else 0

    def scores(n):
        u, b = stages[n]
        b0 = first_block(u)
        for h in range(b * _GB, (b + 1) * _GB):
            v0, off = divmod(h * dh, 16)
            q = _as_i32(q_scr[16 * v0:16 * v0 + 32, 128 * u:128 * (u + 1)])
            wq = []
            for v in range(8):
                slot, half = divmod((v - v0) % 8, 2)
                wq.append(q[8 * half:8 * half + 8] & mask_scr[2 * off + 4 * half + slot])
            p0 = _aligned(step * (_TQ // 2) + (128 * u + _HALO - _W) // 2 + hb * b0, hb)
            s = _dot(_as_bf16(ks_scr[h, pl.ds(p0, hb * (9 - b0)), :]),
                     _as_bf16(jnp.concatenate(wq, axis=0)))
            blocks = [s[_QB * i:_QB * (i + 1)] for i in range(9 - b0)]
            if first:
                for i in range(3):
                    blocks[i] = jnp.where(lane >= 32 * (3 - i), blocks[i], _MASKED)
                blocks[-1] = jnp.where(causal, blocks[-1], _MASKED)
            else:
                blocks = blocks[1:8] + [jnp.where(causal, blocks[8], blocks[0])]
            s = jnp.concatenate(blocks, axis=0)
            s_scr[n % nslot, h % _GB, 0:s.shape[0]] = s
            maxes[u, h] = jnp.max(s, axis=0, keepdims=True)

    def pick(cond, x, y):
        return jnp.where(cond, zero if x is None else x, zero if y is None else y)

    def values(n):
        u, b = stages[n]
        b0 = first_block(u)
        nblk = 9 - b0 if first else 8
        f0 = b0 + 3 if first else 0
        for h in range(b * _GB, (b + 1) * _GB):
            p = _pack_rows(jnp.exp2(s_scr[n % nslot, h % _GB, 0:_QB * nblk] - maxes[u, h]))
            blk = {9 - nblk + i: p[hb * i:hb * (i + 1)] for i in range(nblk)}
            mid = {}
            if not first:
                merged = blk[8]
                blk[0], blk[8] = merged & ~new_bits, merged & new_bits
                mid[0] = merged & jnp.where(odd, 0, ~new_bits)
                mid[9] = merged & jnp.where(odd, new_bits, 0)
            for i in range(max(f0 - 2, 0), 10):
                if i not in mid:
                    mid[i] = pick(odd, blk.get(i - 1), blk.get(i))
            frame = jnp.concatenate(
                [pick(upper, mid.get(i - 2), mid.get(i)) for i in range(f0, 12)], axis=0)
            tile0 = step * (_TQ // 128) + u - _W // 128
            vt = jnp.concatenate(
                [vt_scr[tile0 + c, 32 * h:32 * (h + 1), :] for c in range(f0 // 4, 3)], axis=1)
            r = _dot(vt, _as_bf16(frame))
            ones_row = dh if h % 2 == 0 else 0
            outs[u, h] = r[:24] * (1.0 / r[ones_row:ones_row + 1])
        for c in range(b * _GB * dh // 128, (b + 1) * _GB * dh // 128):
            rows = []
            for v in range(16 * c, 16 * (c + 1)):
                pair, k = divmod(v, 5)
                even, odd_head = outs[u, 2 * pair], outs[u, 2 * pair + 1]
                if k < 2:
                    rows.append(even[8 * k:8 * (k + 1)])
                elif k == 2:
                    rows.append(jnp.where(top4, even[16:], odd_head[:8]))
                else:
                    rows.append(odd_head[8 * (k - 2):8 * (k - 1)])
            att_scr[128 * u:128 * (u + 1), 128 * c:128 * (c + 1)] = (
                jnp.concatenate(rows, axis=0).T.astype(_BF16))

    return len(stages), scores, values


def _kernel(x_hbm, wqkv_hbm, wo_hbm, w1_hbm, b1_hbm, w2_hbm, b2_hbm, o_hbm,
            x_scr, wqkv, wqt, wvt, wo, w1, b1, w2, b2, o_scr, xn_scr, xv_scr, q_scr,
            k_scr, ks_scr, vt_scr, mask_scr, s_scr, att_scr, h_scr, hn_scr, a_scr,
            sems, o_sems):
    s, d = x_scr.shape
    f = w1.shape[-1]
    dh = d // _H
    nsteps = s // _TQ
    cq, ck, cv = (pl.ds(n * d, d) for n in range(3))
    r0, r1, r2 = pl.ds(0, _TQ), pl.ds(_TQ, _TQ), pl.ds(2 * _TQ, s - 2 * _TQ)
    (cp_x0, cp_wk, cp_wq, cp_wv, cp_wo, cp_b1, cp_b2, cp_w1, cp_x1, cp_x2, cp_w2) = [
        pltpu.make_async_copy(src, dst, sems.at[n]) for n, (src, dst) in enumerate(
            [(x_hbm.at[r0], x_scr.at[r0]), (wqkv_hbm.at[:, ck], wqkv.at[:, ck]),
             (wqkv_hbm.at[:, cq], wqkv.at[:, cq]), (wqkv_hbm.at[:, cv], wqkv.at[:, cv]),
             (wo_hbm, wo), (b1_hbm, b1), (b2_hbm, b2), (w1_hbm, w1),
             (x_hbm.at[r1], x_scr.at[r1]), (x_hbm.at[r2], x_scr.at[r2]), (w2_hbm, w2)])]
    top, bottom = slice(0, _TQ // 2), slice(_TQ // 2, _TQ)

    def block_rows(step, r=slice(0, _TQ)):
        return pl.ds(_aligned(step * _TQ + r.start, _TQ // 2), r.stop - r.start)

    def cp_out(step, r=slice(0, _TQ), sem=None):
        rows = block_rows(step, r)
        return pltpu.make_async_copy(
            o_scr.at[rows], o_hbm.at[rows], o_sems.at[step if sem is None else sem])

    def init_tables():
        k_scr[0:_HALO] = jnp.zeros((_HALO, k_scr.shape[1]), _BF16)
        lane = lax.broadcasted_iota(jnp.int32, (8, 128), 1)
        row = lax.broadcasted_iota(jnp.int32, (8, 128), 0)
        for off in range(0, 16, 4):
            for half in range(2):
                feat = 2 * row + (16 * half - off)
                for slot in range(4):
                    mask_scr[2 * off + 4 * half + slot] = jnp.where(
                        (feat >= 0) & (feat < dh) & ((lane >> 5) == slot), -1, 0)

    def pre_norm(step):
        xn = _layernorm(x_scr[block_rows(step)].astype(_F32))
        xn_scr[...] = xn.astype(_BF16)
        xv_scr[...] = _pack_rows(xn)

    def key_proj():
        for m, kt in enumerate(_head_tiles(_dot(xn_scr[...], wqkv[:, ck]))):
            k_scr[_HALO:_HALO + _TQ, 128 * m:128 * (m + 1)] = kt.astype(_BF16)

    def key_slots(step):
        rows = pl.ds(_aligned(step * (_TQ // 2), _TQ // 2), _TQ // 2)
        lane = lax.broadcasted_iota(jnp.int32, (1, 128), 1)
        for m in range(6):
            kt = _as_i32(k_scr[:, 128 * m:128 * (m + 1)])
            slots = [kt[16 * sl:16 * sl + _TQ // 2] for sl in range(4)]
            slots = [pltpu.roll(t, 32 * sl, 1) if sl else t for sl, t in enumerate(slots)]
            for h in range(6 * m, min(6 * m + 6, _H)):
                rel = (lane - h * dh) & 127
                ks_scr[h, rows, :] = jnp.where(
                    rel < 64, jnp.where(rel < 32, slots[0], slots[1]),
                    jnp.where(rel < 96, slots[2], slots[3]))

    def query_proj(first):
        scale = float(dh ** -0.5 * np.log2(np.e))
        qt = _dot(xn_scr[...], wqkv[:, cq]).T if first else _dot(wqt[...], xn_scr[...], _NT)
        q_scr[...] = (qt * scale).astype(_BF16)

    def value_proj(step, first):
        xv = _as_bf16(xv_scr[...])
        vt = _dot(xv, wqkv[:, cv]).T if first else _dot(wvt[...], xv, _NT)
        top4 = lax.broadcasted_iota(jnp.int32, (8, _TQ), 0) < 4
        pieces = []
        for base in range(0, d, 2 * dh):
            shared = vt[base + 16:base + 24]
            pieces += [vt[base:base + 16], jnp.where(top4, shared, 1.0), shared,
                       jnp.where(top4, 1.0, shared), vt[base + 24:base + 40], shared]
        vtp = jnp.concatenate(pieces, axis=0).astype(_BF16)
        for c in range(_TQ // 128):
            vt_scr[step * (_TQ // 128) + c] = vtp[:, 128 * c:128 * (c + 1)]

    def out_proj(step, r):
        h_scr[r] = x_scr[block_rows(step, r)].astype(_F32) + _dot(att_scr[r], wo[...])

    def mid_norm(r):
        hn_scr[r] = _layernorm(h_scr[r]).astype(_BF16)

    def up_proj(r, c):
        cols = slice(c * _FC, (c + 1) * _FC)
        z = _dot(hn_scr[r], w1[:, cols]) + b1[cols].astype(_F32).reshape(1, -1)
        a_scr[r, cols] = _gelu2(z).astype(_BF16)

    def down_proj(step, r):
        y = 0.5 * _dot(a_scr[r], w2[...]) + b2[...].astype(_F32).reshape(1, -1)
        o_scr[block_rows(step, r)] = (h_scr[r] + y).astype(o_scr.dtype)

    def finish(step, early_copy=None):
        mid_norm(bottom)
        down_proj(step, top)
        if early_copy is not None:
            early_copy.start()
        for c in range(f // _FC):
            up_proj(bottom, c)
        down_proj(step, bottom)

    def body(step):
        first = isinstance(step, int)
        if first:
            cp_x0.start()
            cp_wk.start()
            init_tables()
            cp_x0.wait()
            pre_norm(step)
            cp_wq.start()
            cp_wk.wait()
            cp_wv.start()
        else:
            @pl.when(step == 1)
            def _():
                cp_w2.wait()
                cp_x1.wait()
                cp_x2.start()

            pl.when(step == 2)(cp_x2.wait)
            finish(step - 1)
            pre_norm(step)
            k_scr[0:_HALO] = k_scr[_TQ:_TQ + _HALO]
        key_proj()
        if first:
            cp_wq.wait()
            for c in (cp_wo, cp_b1, cp_b2):
                c.start()
        query_proj(first)
        if first:
            cp_wv.wait()
            cp_w1.start()
        key_slots(step)
        value_proj(step, first)

        nb, scores, values = _attention(
            q_scr, ks_scr, vt_scr, mask_scr, s_scr, att_scr, step, dh, first)
        for n in range(nb + _LAG):
            if n < nb:
                scores(n)
            if n == nb - 8:
                if first:
                    for c in (cp_wo, cp_b1, cp_b2, cp_w1):
                        c.wait()
                    cp_w2.start()
                    cp_x1.start()
                out_proj(step, top)
                mid_norm(top)
            if n == nb + 1:
                up_proj(top, 0)
            if n >= _LAG:
                values(n - _LAG)
        if first:
            wqt[...] = wqkv[:, cq].T
            wvt[...] = wqkv[:, cv].T
        for c in range(1, f // _FC):
            up_proj(top, c)
        out_proj(step, bottom)
        if not first:
            cp_out(step - 1).start()

    body(0)
    pl.loop(1, nsteps)(body)
    last = [cp_out(nsteps - 1, top), cp_out(nsteps - 1, bottom, nsteps)]
    finish(nsteps - 1, last[0])
    last[1].start()
    for c in [cp_out(step) for step in range(nsteps - 1)] + last:
        c.wait()


@jax.jit
def pallas_sequential_preLN__sliding_block__dense_activation_gelu__prompt_kernel(
    A_x: jax.Array,
    A_wqkv: jax.Array,
    A_wo: jax.Array,
    B_x: jax.Array,
    B_w1: jax.Array,
    B_b1: jax.Array,
    B_w2: jax.Array,
    B_b2: jax.Array,
):
    del B_x
    b, s, d = A_x.shape
    f = B_w1.shape[1]
    assert b == 1 and d == 640 and s % _TQ == 0 and s >= 3 * _TQ and f % _FC == 0
    hbm = pl.BlockSpec(memory_space=pl.ANY)
    out = pl.pallas_call(
        _kernel,
        in_specs=[hbm] * 7,
        out_specs=hbm,
        out_shape=jax.ShapeDtypeStruct((s, d), A_x.dtype),
        scratch_shapes=[
            pltpu.VMEM((s, d), _BF16),
            pltpu.VMEM((d, 3 * d), _BF16),
            pltpu.VMEM((d, d), _BF16),
            pltpu.VMEM((d, d), _BF16),
            pltpu.VMEM((d, d), _BF16),
            pltpu.VMEM((d, f), _BF16),
            pltpu.VMEM((f,), _BF16),
            pltpu.VMEM((f, d), _BF16),
            pltpu.VMEM((d,), _BF16),
            pltpu.VMEM((s, d), A_x.dtype),
            pltpu.VMEM((_TQ, d), _BF16),
            pltpu.VMEM((_TQ // 2, d), jnp.int32),
            pltpu.VMEM((d, _TQ), _BF16),
            pltpu.VMEM((_HALO + _TQ, 6 * 128), _BF16),
            pltpu.VMEM((_H, s // 2, 128), jnp.int32),
            pltpu.VMEM((s // 128, 32 * _H, 128), _BF16),
            pltpu.VMEM((32, 8, 128), jnp.int32),
            pltpu.VMEM((_LAG + 1, _GB, _W, 128), _F32),
            pltpu.VMEM((_TQ, d), _BF16),
            pltpu.VMEM((_TQ, d), _F32),
            pltpu.VMEM((_TQ, d), _BF16),
            pltpu.VMEM((_TQ, f), _BF16),
            pltpu.SemaphoreType.DMA((11,)),
            pltpu.SemaphoreType.DMA((s // _TQ + 1,)),
        ],
        compiler_params=pltpu.CompilerParams(vmem_limit_bytes=100 * 1024 * 1024),
    )(A_x.reshape(s, d), A_wqkv, A_wo, B_w1, B_b1, B_w2, B_b2)
    return out.reshape(b, s, d)
```

```python
import jax
import jax.numpy as jnp
import numpy as np
from jax import lax
from jax.experimental import pallas as pl
from jax.experimental.pallas import tpu as pltpu

_H = 32
_W = 256
_TQ = 256
_QB = 32
_GB = 2
_LAG = 4
_FC = 384
_HALO = 96
_EPS = 1e-5
_MASKED = -1e30
_F32 = jnp.float32
_BF16 = jnp.bfloat16
_NT = (((1,), (1,)), ((), ()))
_NN = (((1,), (0,)), ((), ()))


def _dot(a, b, dims=_NN):
    return lax.dot_general(a, b, dims, preferred_element_type=_F32)


def _gelu2(x):
    c = float(np.sqrt(2.0 / np.pi))
    return x * jnp.tanh(x * (x * x * (0.044715 * c) + c)) + x


def _layernorm(x):
    m = jnp.mean(x, axis=-1, keepdims=True)
    c = x - m
    v = jnp.mean(c * c, axis=-1, keepdims=True)
    return c * lax.rsqrt(v + _EPS)


def _as_i32(x):
    return pltpu.bitcast(x, jnp.int32)


def _as_bf16(x):
    return pltpu.bitcast(x, _BF16)


def _head_tiles(t):
    tiles = [t[:, 128 * c:128 * (c + 1)] for c in range(5)]
    lane = lax.broadcasted_iota(jnp.int32, (1, 128), 1)
    return ([tiles[0]]
            + [jnp.where(lane >= 128 - 8 * m, tiles[m - 1], tiles[m]) for m in range(1, 5)]
            + [tiles[4]])


def _aligned(i, n):
    return i if isinstance(i, int) else pl.multiple_of(i, n)


def _attention(q_scr, ks_scr, vt_scr, mask_scr, s_scr, att_scr, step, dh, first):
    hb = _QB // 2
    row = lax.broadcasted_iota(jnp.int32, (_QB, 128), 0)
    lane = lax.broadcasted_iota(jnp.int32, (_QB, 128), 1)
    col = lane & (_QB - 1)
    causal = row <= col
    prow = 2 * row[:hb]
    new_bits = (jnp.where(prow <= col[:hb], 0xFFFF, 0)
                | jnp.where(prow + 1 <= col[:hb], -65536, 0))
    odd = (lane[:hb] & 32) != 0
    upper = lane[:hb] >= 64
    top4 = lax.broadcasted_iota(jnp.int32, (8, 128), 0) < 4
    zero = jnp.zeros((hb, 128), jnp.int32)
    nslot = s_scr.shape[0]
    stages = [(u, b) for u in range(_TQ // 128) for b in range(_H // _GB)]
    maxes, outs = {}, {}

    def first_block(u):
        return 5 - 4 * u if first else 0

    def scores(n):
        u, b = stages[n]
        b0 = first_block(u)
        for h in range(b * _GB, (b + 1) * _GB):
            v0, off = divmod(h * dh, 16)
            q = _as_i32(q_scr[16 * v0:16 * v0 + 32, 128 * u:128 * (u + 1)])
            wq = []
            for v in range(8):
                slot, half = divmod((v - v0) % 8, 2)
                wq.append(q[8 * half:8 * half + 8] & mask_scr[2 * off + 4 * half + slot])
            p0 = _aligned(step * (_TQ // 2) + (128 * u + _HALO - _W) // 2 + hb * b0, hb)
            s = _dot(_as_bf16(ks_scr[h, pl.ds(p0, hb * (9 - b0)), :]),
                     _as_bf16(jnp.concatenate(wq, axis=0)))
            blocks = [s[_QB * i:_QB * (i + 1)] for i in range(9 - b0)]
            if first:
                for i in range(3):
                    blocks[i] = jnp.where(lane >= 32 * (3 - i), blocks[i], _MASKED)
                blocks[-1] = jnp.where(causal, blocks[-1], _MASKED)
            else:
                blocks = blocks[1:8] + [jnp.where(causal, blocks[8], blocks[0])]
            s = jnp.concatenate(blocks, axis=0)
            s_scr[n % nslot, h % _GB, 0:s.shape[0]] = s
            maxes[u, h] = jnp.max(s, axis=0, keepdims=True)

    def pick(cond, x, y):
        return jnp.where(cond, zero if x is None else x, zero if y is None else y)

    def values(n):
        u, b = stages[n]
        b0 = first_block(u)
        nblk = 9 - b0 if first else 8
        f0 = b0 + 3 if first else 0
        for h in range(b * _GB, (b + 1) * _GB):
            p = jnp.exp2(s_scr[n % nslot, h % _GB, 0:_QB * nblk] - maxes[u, h])
            p = _as_i32(p.astype(_BF16))
            blk = {9 - nblk + i: p[hb * i:hb * (i + 1)] for i in range(nblk)}
            mid = {}
            if not first:
                merged = blk[8]
                blk[0], blk[8] = merged & ~new_bits, merged & new_bits
                mid[0] = merged & jnp.where(odd, 0, ~new_bits)
                mid[9] = merged & jnp.where(odd, new_bits, 0)
            for i in range(max(f0 - 2, 0), 10):
                if i not in mid:
                    mid[i] = pick(odd, blk.get(i - 1), blk.get(i))
            frame = jnp.concatenate(
                [pick(upper, mid.get(i - 2), mid.get(i)) for i in range(f0, 12)], axis=0)
            tile0 = step * (_TQ // 128) + u - _W // 128
            vt = jnp.concatenate(
                [vt_scr[tile0 + c, 32 * h:32 * (h + 1), :] for c in range(f0 // 4, 3)], axis=1)
            r = _dot(vt, _as_bf16(frame))
            ones_row = dh if h % 2 == 0 else 0
            outs[u, h] = r[:24] * (1.0 / r[ones_row:ones_row + 1])
        for c in range(b * _GB * dh // 128, (b + 1) * _GB * dh // 128):
            rows = []
            for v in range(16 * c, 16 * (c + 1)):
                pair, k = divmod(v, 5)
                even, odd_head = outs[u, 2 * pair], outs[u, 2 * pair + 1]
                if k < 2:
                    rows.append(even[8 * k:8 * (k + 1)])
                elif k == 2:
                    rows.append(jnp.where(top4, even[16:], odd_head[:8]))
                else:
                    rows.append(odd_head[8 * (k - 2):8 * (k - 1)])
            att_scr[128 * u:128 * (u + 1), 128 * c:128 * (c + 1)] = (
                jnp.concatenate(rows, axis=0).T.astype(_BF16))

    return len(stages), scores, values


def _kernel(x_hbm, wqkv_hbm, wo_hbm, w1_hbm, b1_hbm, w2_hbm, b2_hbm, o_hbm,
            x_scr, wqkv, wqt, wvt, wo, w1, b1, w2, b2, o_scr, xn_scr, q_scr,
            k_scr, ks_scr, vt_scr, mask_scr, s_scr, att_scr, h_scr, hn_scr, a_scr,
            sems, o_sems):
    s, d = x_scr.shape
    f = w1.shape[-1]
    dh = d // _H
    nsteps = s // _TQ
    cq, ck, cv = (pl.ds(n * d, d) for n in range(3))
    r0, r1, r2 = pl.ds(0, _TQ), pl.ds(_TQ, _TQ), pl.ds(2 * _TQ, s - 2 * _TQ)
    (cp_x0, cp_wk, cp_wq, cp_wv, cp_wo, cp_b1, cp_b2, cp_w1, cp_x1, cp_x2, cp_w2) = [
        pltpu.make_async_copy(src, dst, sems.at[n]) for n, (src, dst) in enumerate(
            [(x_hbm.at[r0], x_scr.at[r0]), (wqkv_hbm.at[:, ck], wqkv.at[:, ck]),
             (wqkv_hbm.at[:, cq], wqkv.at[:, cq]), (wqkv_hbm.at[:, cv], wqkv.at[:, cv]),
             (wo_hbm, wo), (b1_hbm, b1), (b2_hbm, b2), (w1_hbm, w1),
             (x_hbm.at[r1], x_scr.at[r1]), (x_hbm.at[r2], x_scr.at[r2]), (w2_hbm, w2)])]
    top, bottom = slice(0, _TQ // 2), slice(_TQ // 2, _TQ)

    def block_rows(step, r=slice(0, _TQ)):
        return pl.ds(_aligned(step * _TQ + r.start, _TQ // 2), r.stop - r.start)

    def cp_out(step, r=slice(0, _TQ), sem=None):
        rows = block_rows(step, r)
        return pltpu.make_async_copy(
            o_scr.at[rows], o_hbm.at[rows], o_sems.at[step if sem is None else sem])

    def init_tables():
        k_scr[0:_HALO] = jnp.zeros((_HALO, k_scr.shape[1]), _BF16)
        lane = lax.broadcasted_iota(jnp.int32, (8, 128), 1)
        row = lax.broadcasted_iota(jnp.int32, (8, 128), 0)
        for off in range(0, 16, 4):
            for half in range(2):
                feat = 2 * row + (16 * half - off)
                for slot in range(4):
                    mask_scr[2 * off + 4 * half + slot] = jnp.where(
                        (feat >= 0) & (feat < dh) & ((lane >> 5) == slot), -1, 0)

    def pre_norm(step):
        xn_scr[...] = _layernorm(x_scr[block_rows(step)].astype(_F32)).astype(_BF16)

    def key_proj():
        for m, kt in enumerate(_head_tiles(_dot(xn_scr[...], wqkv[:, ck]))):
            k_scr[_HALO:_HALO + _TQ, 128 * m:128 * (m + 1)] = kt.astype(_BF16)

    def key_slots(step):
        rows = pl.ds(_aligned(step * (_TQ // 2), _TQ // 2), _TQ // 2)
        lane = lax.broadcasted_iota(jnp.int32, (1, 128), 1)
        for m in range(6):
            kt = _as_i32(k_scr[:, 128 * m:128 * (m + 1)])
            slots = [kt[16 * sl:16 * sl + _TQ // 2] for sl in range(4)]
            slots = [pltpu.roll(t, 32 * sl, 1) if sl else t for sl, t in enumerate(slots)]
            for h in range(6 * m, min(6 * m + 6, _H)):
                rel = (lane - h * dh) & 127
                ks_scr[h, rows, :] = jnp.where(
                    rel < 64, jnp.where(rel < 32, slots[0], slots[1]),
                    jnp.where(rel < 96, slots[2], slots[3]))

    def query_proj(first):
        scale = float(dh ** -0.5 * np.log2(np.e))
        qt = _dot(xn_scr[...], wqkv[:, cq]).T if first else _dot(wqt[...], xn_scr[...], _NT)
        q_scr[...] = (qt * scale).astype(_BF16)

    def value_proj(step, first):
        vt = _dot(xn_scr[...], wqkv[:, cv]).T if first else _dot(wvt[...], xn_scr[...], _NT)
        top4 = lax.broadcasted_iota(jnp.int32, (8, _TQ), 0) < 4
        pieces = []
        for base in range(0, d, 2 * dh):
            shared = vt[base + 16:base + 24]
            pieces += [vt[base:base + 16], jnp.where(top4, shared, 1.0), shared,
                       jnp.where(top4, 1.0, shared), vt[base + 24:base + 40], shared]
        vtp = jnp.concatenate(pieces, axis=0).astype(_BF16)
        for c in range(_TQ // 128):
            vt_scr[step * (_TQ // 128) + c] = vtp[:, 128 * c:128 * (c + 1)]

    def out_proj(step, r):
        h_scr[r] = x_scr[block_rows(step, r)].astype(_F32) + _dot(att_scr[r], wo[...])

    def mid_norm(r):
        hn_scr[r] = _layernorm(h_scr[r]).astype(_BF16)

    def up_proj(r, c):
        cols = slice(c * _FC, (c + 1) * _FC)
        z = _dot(hn_scr[r], w1[:, cols]) + b1[cols].astype(_F32).reshape(1, -1)
        a_scr[r, cols] = _gelu2(z).astype(_BF16)

    def down_proj(step, r):
        y = 0.5 * _dot(a_scr[r], w2[...]) + b2[...].astype(_F32).reshape(1, -1)
        o_scr[block_rows(step, r)] = (h_scr[r] + y).astype(o_scr.dtype)

    def finish(step, early_copy=None):
        mid_norm(bottom)
        down_proj(step, top)
        if early_copy is not None:
            early_copy.start()
        for c in range(f // _FC):
            up_proj(bottom, c)
        down_proj(step, bottom)

    def body(step):
        first = isinstance(step, int)
        if first:
            cp_x0.start()
            cp_wk.start()
            init_tables()
            cp_x0.wait()
            pre_norm(step)
            cp_wq.start()
            cp_wk.wait()
            cp_wv.start()
        else:
            @pl.when(step == 1)
            def _():
                cp_w2.wait()
                cp_x1.wait()
                cp_x2.start()

            pl.when(step == 2)(cp_x2.wait)
            finish(step - 1)
            pre_norm(step)
            k_scr[0:_HALO] = k_scr[_TQ:_TQ + _HALO]
        key_proj()
        if first:
            cp_wq.wait()
            for c in (cp_wo, cp_b1, cp_b2):
                c.start()
        query_proj(first)
        if first:
            cp_wv.wait()
            cp_w1.start()
        key_slots(step)
        value_proj(step, first)

        nb, scores, values = _attention(
            q_scr, ks_scr, vt_scr, mask_scr, s_scr, att_scr, step, dh, first)
        for n in range(nb + _LAG):
            if n < nb:
                scores(n)
            if n == nb - 8:
                if first:
                    for c in (cp_wo, cp_b1, cp_b2, cp_w1):
                        c.wait()
                    cp_w2.start()
                    cp_x1.start()
                out_proj(step, top)
                mid_norm(top)
            if n == nb + 1:
                up_proj(top, 0)
            if n >= _LAG:
                values(n - _LAG)
        if first:
            wqt[...] = wqkv[:, cq].T
            wvt[...] = wqkv[:, cv].T
        for c in range(1, f // _FC):
            up_proj(top, c)
        out_proj(step, bottom)
        if not first:
            cp_out(step - 1).start()

    body(0)
    pl.loop(1, nsteps)(body)
    last = [cp_out(nsteps - 1, top), cp_out(nsteps - 1, bottom, nsteps)]
    finish(nsteps - 1, last[0])
    last[1].start()
    for c in [cp_out(step) for step in range(nsteps - 1)] + last:
        c.wait()


@jax.jit
def pallas_sequential_preLN__sliding_block__dense_activation_gelu__prompt_kernel(
    A_x: jax.Array,
    A_wqkv: jax.Array,
    A_wo: jax.Array,
    B_x: jax.Array,
    B_w1: jax.Array,
    B_b1: jax.Array,
    B_w2: jax.Array,
    B_b2: jax.Array,
):
    del B_x
    b, s, d = A_x.shape
    f = B_w1.shape[1]
    assert b == 1 and d == 640 and s % _TQ == 0 and s >= 3 * _TQ and f % _FC == 0
    hbm = pl.BlockSpec(memory_space=pl.ANY)
    out = pl.pallas_call(
        _kernel,
        in_specs=[hbm] * 7,
        out_specs=hbm,
        out_shape=jax.ShapeDtypeStruct((s, d), A_x.dtype),
        scratch_shapes=[
            pltpu.VMEM((s, d), _BF16),
            pltpu.VMEM((d, 3 * d), _BF16),
            pltpu.VMEM((d, d), _BF16),
            pltpu.VMEM((d, d), _BF16),
            pltpu.VMEM((d, d), _BF16),
            pltpu.VMEM((d, f), _BF16),
            pltpu.VMEM((f,), _BF16),
            pltpu.VMEM((f, d), _BF16),
            pltpu.VMEM((d,), _BF16),
            pltpu.VMEM((s, d), A_x.dtype),
            pltpu.VMEM((_TQ, d), _BF16),
            pltpu.VMEM((d, _TQ), _BF16),
            pltpu.VMEM((_HALO + _TQ, 6 * 128), _BF16),
            pltpu.VMEM((_H, s // 2, 128), jnp.int32),
            pltpu.VMEM((s // 128, 32 * _H, 128), _BF16),
            pltpu.VMEM((32, 8, 128), jnp.int32),
            pltpu.VMEM((_LAG + 1, _GB, _W, 128), _F32),
            pltpu.VMEM((_TQ, d), _BF16),
            pltpu.VMEM((_TQ, d), _F32),
            pltpu.VMEM((_TQ, d), _BF16),
            pltpu.VMEM((_TQ, f), _BF16),
            pltpu.SemaphoreType.DMA((11,)),
            pltpu.SemaphoreType.DMA((s // _TQ + 1,)),
        ],
        compiler_params=pltpu.CompilerParams(vmem_limit_bytes=100 * 1024 * 1024),
    )(A_x.reshape(s, d), A_wqkv, A_wo, B_w1, B_b1, B_w2, B_b2)
    return out.reshape(b, s, d)
```
